```python
import os as _os
_os.environ.setdefault("JAX_PLATFORMS", "cpu")
import jax
import jax.numpy as jnp

def _softmax(x, axis=-1):
    return jax.nn.softmax(x, axis=axis)
def _gelu(x):
    return jax.nn.gelu(x, approximate=True)
def _silu(x):
    return jax.nn.silu(x)
def _sigmoid(x):
    return jax.nn.sigmoid(x)
def _layernorm(x, axis=-1, eps=1e-5):
    m = jnp.mean(x, axis=axis, keepdims=True)
    v = jnp.var(x, axis=axis, keepdims=True)
    return (x - m) / jnp.sqrt(v + eps)
def _scatter_add(tgt, idx, src, axis=0):
    return tgt.at[idx].add(src)
def _segment_sum(src, seg, n):
    return jax.ops.segment_sum(src, seg, n)
class _Rng:
    def __init__(self, key):
        self._k = key
    def _next(self):
        self._k, sub = jax.random.split(self._k)
        return sub
    def normal(self, shape):
        return jax.random.normal(self._next(), shape, dtype=jnp.bfloat16)
    def randint(self, lo, hi, shape):
        return jax.random.randint(self._next(), shape, lo, hi, dtype=jnp.int32)
    def uniform(self, shape, lo=0.0, hi=1.0):
        return jax.random.uniform(self._next(), shape, jnp.bfloat16, lo, hi)
    def permutation(self, n):
        return jax.random.permutation(self._next(), n)


kernel_name = 'standalone__mha_softmax__sampling'

def setup_inputs():
    _rng = _Rng(jax.random.key(int.from_bytes(__import__("os").urandom(4), "little")))
    _w = (lambda a: (lambda t: t.astype(jnp.bfloat16) if jnp.issubdtype(t.dtype, jnp.floating) else t)(jnp.asarray(a)))
    B, H, Sq, Sk, D = 8, 32, 8, 4096, 128
    return {
        "q": _w((lambda *s: _rng.normal(s) * 0.4)(B, H, Sq, D)),
        "k": _w((lambda *s: _rng.normal(s) * 0.4)(B, H, Sk, D)),
        "v": _w((lambda *s: _rng.normal(s) * 0.05)(B, H, Sk, D)),
    }

def reference(q, k, v):
    scale = q.shape[-1] ** -0.5
    scores = jnp.einsum("bhqd,bhkd->bhqk", q, k) * scale
    p = _softmax(scores, axis=-1)
    return jnp.einsum("bhqk,bhkd->bhqd", p, v)
```

```python
import functools

import jax
import jax.numpy as jnp
from jax import lax
import jax.experimental.pallas as pl
import jax.experimental.pallas.tpu as pltpu

HB = 2


def _kernel(q_ref, k_ref, v_ref, o_ref, *, scale):
    for h in range(HB):
        q = q_ref[h]
        k = k_ref[h]
        s = lax.dot_general(q, k, (((1,), (1,)), ((), ())),
                            preferred_element_type=jnp.float32) * scale
        m = jnp.max(s, axis=-1, keepdims=True)
        p = jnp.exp(s - m)
        l = jnp.sum(p, axis=-1, keepdims=True)
        o = jnp.dot(p.astype(jnp.bfloat16), v_ref[h],
                    preferred_element_type=jnp.float32)
        o_ref[h] = (o / l).astype(o_ref.dtype)


@jax.jit
def pallas_standalone__mha_softmax__sampling_kernel(q, k, v):
    B, H, Sq, D = q.shape
    Sk = k.shape[2]
    BH = B * H
    qf = q.reshape(BH, Sq, D)
    kf = k.reshape(BH, Sk, D)
    vf = v.reshape(BH, Sk, D)
    out = pl.pallas_call(
        functools.partial(_kernel, scale=D ** -0.5),
        grid=(BH // HB,),
        in_specs=[
            pl.BlockSpec((HB, Sq, D), lambda i: (i, 0, 0)),
            pl.BlockSpec((HB, Sk, D), lambda i: (i, 0, 0)),
            pl.BlockSpec((HB, Sk, D), lambda i: (i, 0, 0)),
        ],
        out_specs=pl.BlockSpec((HB, Sq, D), lambda i: (i, 0, 0)),
        out_shape=jax.ShapeDtypeStruct((BH, Sq, D), q.dtype),
        compiler_params=pltpu.CompilerParams(
            dimension_semantics=("arbitrary",),
            vmem_limit_bytes=64 * 1024 * 1024,
        ),
    )(qf, kf, vf)
    return out.reshape(B, H, Sq, D)
```

```python
import math

import jax
import jax.numpy as jnp
from jax import lax
import jax.experimental.pallas as pl
import jax.experimental.pallas.tpu as pltpu

LOG2E = math.log2(math.e)

NH = 8
C = 512
P = 16
S = 3


def _make_kernel(NG, NC, Sk, D):
    NSTEP = NG * NC
    NP = C // P
    c_scale = (D ** -0.5) * LOG2E

    def kernel(q_hbm, k_hbm, v_hbm, o_hbm, qbuf, kbuf, vbuf, obuf,
               m_ref, l_ref, acc_ref, qsem, ksem, vsem, osem):
        def start_chunk(step):
            g = step // NC
            c = lax.rem(step, NC)
            slot = lax.rem(step, S)
            for j in range(NP):
                off = pl.multiple_of(c * C + j * P, P)
                pltpu.make_async_copy(
                    k_hbm.at[g, :, pl.ds(off, P)],
                    kbuf.at[slot, :, pl.ds(j * P, P)],
                    ksem.at[slot]).start(priority=0)
                pltpu.make_async_copy(
                    v_hbm.at[g, :, pl.ds(off, P)],
                    vbuf.at[slot, :, pl.ds(j * P, P)],
                    vsem.at[slot]).start(priority=1)

        qcopy = pltpu.make_async_copy(q_hbm, qbuf, qsem)
        qcopy.start()
        for i in range(S - 1):
            start_chunk(i)
        qcopy.wait()

        def body(step, carry):
            g = step // NC
            c = lax.rem(step, NC)
            slot = lax.rem(step, S)

            @pl.when(step + S - 1 < NSTEP)
            def _():
                start_chunk(step + S - 1)

            @pl.when(c == 0)
            def _():
                m_ref[...] = jnp.full(m_ref.shape, -1e30, jnp.float32)
                l_ref[...] = jnp.zeros(l_ref.shape, jnp.float32)
                acc_ref[...] = jnp.zeros(acc_ref.shape, jnp.float32)

            pltpu.make_async_copy(kbuf.at[slot], kbuf.at[slot], ksem.at[slot]).wait()
            pltpu.make_async_copy(vbuf.at[slot], vbuf.at[slot], vsem.at[slot]).wait()

            for h in range(NH):
                q = qbuf[g, h]
                k = kbuf[slot, h]
                t = lax.dot_general(q, k, (((1,), (1,)), ((), ())),
                                    preferred_element_type=jnp.float32) * c_scale
                m_old = m_ref[h]
                m_cur = jnp.max(t, axis=-1, keepdims=True)
                m_new = jnp.maximum(m_old, m_cur)
                alpha = jnp.exp2(m_old - m_new)
                p = jnp.exp2(t - m_new[:, 0:1])
                psum = p[:, 0:128]
                for j in range(1, C // 128):
                    psum = psum + p[:, j * 128:(j + 1) * 128]
                l_ref[h] = alpha * l_ref[h] + psum
                pv = jnp.dot(p.astype(jnp.bfloat16), vbuf[slot, h],
                             preferred_element_type=jnp.float32)
                acc_ref[h] = alpha * acc_ref[h] + pv
                m_ref[h] = m_new

            @pl.when(c == NC - 1)
            def _():
                oslot = lax.rem(g, 2)

                @pl.when(g >= 2)
                def _():
                    pltpu.make_async_copy(obuf.at[oslot], o_hbm.at[g - 2],
                                          osem.at[oslot]).wait()
                for h in range(NH):
                    l = jnp.sum(l_ref[h], axis=-1, keepdims=True)
                    obuf[oslot, h] = (acc_ref[h] / l).astype(obuf.dtype)
                pltpu.make_async_copy(obuf.at[oslot], o_hbm.at[g],
                                      osem.at[oslot]).start()
            return carry

        lax.fori_loop(0, NSTEP, body, 0)
        for g in (NG - 2, NG - 1):
            pltpu.make_async_copy(obuf.at[g % 2], o_hbm.at[g],
                                  osem.at[g % 2]).wait()

    return kernel


@jax.jit
def pallas_standalone__mha_softmax__sampling_kernel(q, k, v):
    B, H, Sq, D = q.shape
    Sk = k.shape[2]
    NG = (B * H) // NH
    NC = Sk // C
    qf = q.reshape(NG, NH, Sq, D)
    kf = k.reshape(NG, NH, Sk, D)
    vf = v.reshape(NG, NH, Sk, D)
    out = pl.pallas_call(
        _make_kernel(NG, NC, Sk, D),
        in_specs=[pl.BlockSpec(memory_space=pl.ANY)] * 3,
        out_specs=pl.BlockSpec(memory_space=pl.ANY),
        out_shape=jax.ShapeDtypeStruct((NG, NH, Sq, D), q.dtype),
        scratch_shapes=[
            pltpu.VMEM((NG, NH, Sq, D), jnp.bfloat16),
            pltpu.VMEM((S, NH, C, D), jnp.bfloat16),
            pltpu.VMEM((S, NH, C, D), jnp.bfloat16),
            pltpu.VMEM((2, NH, Sq, D), jnp.bfloat16),
            pltpu.VMEM((NH, Sq, 128), jnp.float32),
            pltpu.VMEM((NH, Sq, 128), jnp.float32),
            pltpu.VMEM((NH, Sq, D), jnp.float32),
            pltpu.SemaphoreType.DMA(()),
            pltpu.SemaphoreType.DMA((S,)),
            pltpu.SemaphoreType.DMA((S,)),
            pltpu.SemaphoreType.DMA((2,)),
        ],
        compiler_params=pltpu.CompilerParams(
            vmem_limit_bytes=100 * 1024 * 1024,
            disable_bounds_checks=True,
        ),
    )(qf, kf, vf)
    return out.reshape(B, H, Sq, D)
```

```python
import math

import jax
import jax.numpy as jnp
from jax import lax
import jax.experimental.pallas as pl
import jax.experimental.pallas.tpu as pltpu

LOG2E = math.log2(math.e)

NH = 8
C = 256
P = 16
S = 5


def _make_kernel(NG, NC, D):
    NSTEP = NG * NC
    NP = C // P
    c_scale = (D ** -0.5) * LOG2E

    def kernel(q_hbm, k_hbm, v_hbm, o_hbm, qbuf, kbuf, vbuf, obuf,
               m_ref, l_ref, acc_ref, qsem, kvsem, osem):
        def start_chunk(step):
            g = step // NC
            c = lax.rem(step, NC)
            slot = lax.rem(step, S)
            for j in range(NP):
                off = pl.multiple_of(c * C + j * P, P)
                pltpu.make_async_copy(
                    k_hbm.at[g, :, pl.ds(off, P)],
                    kbuf.at[slot, :, pl.ds(j * P, P)],
                    kvsem.at[slot, 0]).start(priority=0)
                pltpu.make_async_copy(
                    v_hbm.at[g, :, pl.ds(off, P)],
                    vbuf.at[slot, :, pl.ds(j * P, P)],
                    kvsem.at[slot, 1]).start(priority=1)

        qcopy = pltpu.make_async_copy(q_hbm, qbuf, qsem)
        qcopy.start()
        for i in range(S - 1):
            start_chunk(i)
        qcopy.wait()

        bulk = pltpu.make_async_copy(obuf.at[pl.ds(0, NG - 1)],
                                     o_hbm.at[pl.ds(0, NG - 1)], osem.at[0])

        def body(step, carry):
            g = step // NC
            c = lax.rem(step, NC)
            slot = lax.rem(step, S)

            @pl.when(step + S - 1 < NSTEP)
            def _():
                start_chunk(step + S - 1)

            @pl.when(step == NSTEP - 1)
            def _():
                bulk.start()

            @pl.when(c == 0)
            def _():
                m_ref[...] = jnp.full(m_ref.shape, -1e30, jnp.float32)
                l_ref[...] = jnp.zeros(l_ref.shape, jnp.float32)
                acc_ref[...] = jnp.zeros(acc_ref.shape, jnp.float32)

            pltpu.make_async_copy(kbuf.at[slot], kbuf.at[slot],
                                  kvsem.at[slot, 0]).wait()

            q = qbuf[g]
            t = lax.dot_general(q, kbuf[slot], (((2,), (2,)), ((0,), (0,))),
                                preferred_element_type=jnp.float32) * c_scale
            m_old = m_ref[...]
            m_new = jnp.maximum(m_old, jnp.max(t, axis=-1, keepdims=True))
            alpha = jnp.exp2(m_old - m_new)
            p = jnp.exp2(t - m_new[:, :, 0:1])
            psum = p[:, :, 0:128]
            for j in range(1, C // 128):
                psum = psum + p[:, :, j * 128:(j + 1) * 128]
            l_ref[...] = alpha * l_ref[...] + psum
            m_ref[...] = m_new
            pb = p.astype(jnp.bfloat16)

            pltpu.make_async_copy(vbuf.at[slot], vbuf.at[slot],
                                  kvsem.at[slot, 1]).wait()
            pv = lax.dot_general(pb, vbuf[slot], (((2,), (1,)), ((0,), (0,))),
                                 preferred_element_type=jnp.float32)
            acc_ref[...] = alpha * acc_ref[...] + pv

            @pl.when(c == NC - 1)
            def _():
                l = jnp.sum(l_ref[...], axis=-1, keepdims=True)
                obuf[g] = (acc_ref[...] / l).astype(obuf.dtype)
            return carry

        lax.fori_loop(0, NSTEP, body, 0)
        last = pltpu.make_async_copy(obuf.at[NG - 1], o_hbm.at[NG - 1], osem.at[1])
        last.start(priority=1)
        bulk.wait()
        last.wait()

    return kernel


@jax.jit
def pallas_standalone__mha_softmax__sampling_kernel(q, k, v):
    B, H, Sq, D = q.shape
    Sk = k.shape[2]
    NG = (B * H) // NH
    NC = Sk // C
    qf = q.reshape(NG, NH, Sq, D)
    kf = k.reshape(NG, NH, Sk, D)
    vf = v.reshape(NG, NH, Sk, D)
    out = pl.pallas_call(
        _make_kernel(NG, NC, D),
        in_specs=[pl.BlockSpec(memory_space=pl.ANY)] * 3,
        out_specs=pl.BlockSpec(memory_space=pl.ANY),
        out_shape=jax.ShapeDtypeStruct((NG, NH, Sq, D), q.dtype),
        scratch_shapes=[
            pltpu.VMEM((NG, NH, Sq, D), jnp.bfloat16),
            pltpu.VMEM((S, NH, C, D), jnp.bfloat16),
            pltpu.VMEM((S, NH, C, D), jnp.bfloat16),
            pltpu.VMEM((NG, NH, Sq, D), jnp.bfloat16),
            pltpu.VMEM((NH, Sq, 128), jnp.float32),
            pltpu.VMEM((NH, Sq, 128), jnp.float32),
            pltpu.VMEM((NH, Sq, D), jnp.float32),
            pltpu.SemaphoreType.DMA(()),
            pltpu.SemaphoreType.DMA((S, 2)),
            pltpu.SemaphoreType.DMA((2,)),
        ],
        compiler_params=pltpu.CompilerParams(
            vmem_limit_bytes=64 * 1024 * 1024,
            disable_bounds_checks=True,
        ),
    )(qf, kf, vf)
    return out.reshape(B, H, Sq, D)
```

```python
import math

import jax
import jax.numpy as jnp
from jax import lax
import jax.experimental.pallas as pl
import jax.experimental.pallas.tpu as pltpu

LOG2E = math.log2(math.e)

NH = 16
C = 128
P = 8
S = 5
L = 6


def _make_kernel(NG, NC, D):
    NSTEP = NG * NC
    NP = C // P
    c_scale = (D ** -0.5) * LOG2E

    def kernel(q_hbm, k_hbm, v_hbm, o_hbm, qbuf, kbuf, vbuf, obuf,
               m_ref, l_ref, acc_ref, qsem, kvsem, osem):
        def coords(s):
            return s // NC, lax.rem(s, NC), lax.rem(s, S)

        def kstart(g, c, slot, j):
            off = pl.multiple_of(c * C + j * P, P)
            pltpu.make_async_copy(
                k_hbm.at[g, :, pl.ds(off, P)],
                kbuf.at[slot, :, pl.ds(j * P, P)],
                kvsem.at[slot, 0]).start(priority=0)

        def vstart(g, c, slot, j):
            off = pl.multiple_of(c * C + j * P, P)
            pltpu.make_async_copy(
                v_hbm.at[g, :, pl.ds(off, P)],
                vbuf.at[slot, :, pl.ds(j * P, P)],
                kvsem.at[slot, 1]).start(priority=1)

        def issue(s, first=False):
            cur = coords(s)
            prev = None if first else coords(s - 1)
            for j in range(NP):
                kstart(*cur, j)
                i = j - L
                if i >= 0:
                    vstart(*cur, i)
                elif not first:
                    vstart(*prev, NP + i)

        def issue_tail():
            s = NSTEP - 1
            g, c, slot = s // NC, s % NC, s % S
            for i in range(NP - L, NP):
                vstart(g, c, slot, i)

        qcopy = pltpu.make_async_copy(q_hbm, qbuf, qsem)
        qcopy.start()
        for i in range(S - 1):
            issue(i, first=(i == 0))
        qcopy.wait()

        bulk = pltpu.make_async_copy(obuf.at[pl.ds(0, NG - 1)],
                                     o_hbm.at[pl.ds(0, NG - 1)], osem.at[0])

        def body(step, carry):
            g = step // NC
            c = lax.rem(step, NC)
            slot = lax.rem(step, S)

            @pl.when(step + S - 1 < NSTEP)
            def _():
                issue(step + S - 1)

            @pl.when(step + S - 1 == NSTEP)
            def _():
                issue_tail()

            @pl.when(c == 0)
            def _():
                m_ref[...] = jnp.full(m_ref.shape, -jnp.inf, jnp.float32)
                l_ref[...] = jnp.zeros(l_ref.shape, jnp.float32)
                acc_ref[...] = jnp.zeros(acc_ref.shape, jnp.float32)

            pltpu.make_async_copy(kbuf.at[slot], kbuf.at[slot],
                                  kvsem.at[slot, 0]).wait()

            @pl.when(step == NSTEP - 1)
            def _():
                bulk.start()

            q = qbuf[g]
            t = lax.dot_general(q, kbuf[slot], (((2,), (2,)), ((0,), (0,))),
                                preferred_element_type=jnp.float32) * c_scale
            m_old = m_ref[...]
            m_new = jnp.maximum(m_old, jnp.max(t, axis=-1, keepdims=True))
            alpha = jnp.exp2(m_old - m_new)
            p = jnp.exp2(t - m_new[:, :, 0:1])
            psum = p[:, :, 0:128]
            for j in range(1, C // 128):
                psum = psum + p[:, :, j * 128:(j + 1) * 128]
            l_ref[...] = alpha * l_ref[...] + psum
            m_ref[...] = m_new
            pb = p.astype(jnp.bfloat16)

            pltpu.make_async_copy(vbuf.at[slot], vbuf.at[slot],
                                  kvsem.at[slot, 1]).wait()
            pv = lax.dot_general(pb, vbuf[slot], (((2,), (1,)), ((0,), (0,))),
                                 preferred_element_type=jnp.float32)
            acc_ref[...] = alpha * acc_ref[...] + pv

            @pl.when(c == NC - 1)
            def _():
                l = jnp.sum(l_ref[...], axis=-1, keepdims=True)
                obuf[g] = (acc_ref[...] / l).astype(obuf.dtype)
            return carry

        lax.fori_loop(0, NSTEP, body, 0)
        last = pltpu.make_async_copy(obuf.at[NG - 1], o_hbm.at[NG - 1], osem.at[1])
        last.start()
        bulk.wait()
        last.wait()

    return kernel


@jax.jit
def pallas_standalone__mha_softmax__sampling_kernel(q, k, v):
    B, H, Sq, D = q.shape
    Sk = k.shape[2]
    NG = (B * H) // NH
    NC = Sk // C
    qf = q.reshape(NG, NH, Sq, D)
    kf = k.reshape(NG, NH, Sk, D)
    vf = v.reshape(NG, NH, Sk, D)
    out = pl.pallas_call(
        _make_kernel(NG, NC, D),
        in_specs=[pl.BlockSpec(memory_space=pl.ANY)] * 3,
        out_specs=pl.BlockSpec(memory_space=pl.ANY),
        out_shape=jax.ShapeDtypeStruct((NG, NH, Sq, D), q.dtype),
        scratch_shapes=[
            pltpu.VMEM((NG, NH, Sq, D), jnp.bfloat16),
            pltpu.VMEM((S, NH, C, D), jnp.bfloat16),
            pltpu.VMEM((S, NH, C, D), jnp.bfloat16),
            pltpu.VMEM((NG, NH, Sq, D), jnp.bfloat16),
            pltpu.VMEM((NH, Sq, 128), jnp.float32),
            pltpu.VMEM((NH, Sq, 128), jnp.float32),
            pltpu.VMEM((NH, Sq, D), jnp.float32),
            pltpu.SemaphoreType.DMA(()),
            pltpu.SemaphoreType.DMA((S, 2)),
            pltpu.SemaphoreType.DMA((2,)),
        ],
        compiler_params=pltpu.CompilerParams(
            vmem_limit_bytes=64 * 1024 * 1024,
            disable_bounds_checks=True,
        ),
    )(qf, kf, vf)
    return out.reshape(B, H, Sq, D)
```
